```python
import jax
import jax.numpy as jnp

def _softmax(x, axis=-1):
    return jax.nn.softmax(x, axis=axis)
def _gelu(x):
    return jax.nn.gelu(x, approximate=True)
def _silu(x):
    return jax.nn.silu(x)
def _sigmoid(x):
    return jax.nn.sigmoid(x)
def _layernorm(x, axis=-1, eps=1e-5):
    m = jnp.mean(x, axis=axis, keepdims=True)
    v = jnp.var(x, axis=axis, keepdims=True)
    return (x - m) / jnp.sqrt(v + eps)
def _scatter_add(tgt, idx, src, axis=0):
    return tgt.at[idx].add(src)
def _segment_sum(src, seg, n):
    return jax.ops.segment_sum(src, seg, n)
class _Rng:
    def __init__(self, key):
        self._k = key
    def _next(self):
        self._k, sub = jax.random.split(self._k)
        return sub
    def normal(self, shape):
        return jax.random.normal(self._next(), shape, dtype=jnp.bfloat16)
    def randint(self, lo, hi, shape):
        return jax.random.randint(self._next(), shape, lo, hi, dtype=jnp.int32)
    def uniform(self, shape, lo=0.0, hi=1.0):
        return jax.random.uniform(self._next(), shape, jnp.bfloat16, lo, hi)
    def permutation(self, n):
        return jax.random.permutation(self._next(), n)


kernel_name = 'standalone__depthwise_separable__vision'

def setup_inputs():
    _rng = _Rng(jax.random.key(int.from_bytes(__import__("os").urandom(4), "little")))
    _w = (lambda a: (lambda t: t.astype(jnp.bfloat16) if jnp.issubdtype(t.dtype, jnp.floating) else t)(jnp.asarray(a)))
    H = W = 384
    C = 384
    k = 1
    return {
        "x": _w((lambda *s: _rng.normal(s) * 0.05)(1, H, W, C)),
        "dw": _w((lambda *s: _rng.normal(s) * 0.05)(k, k, C)),
        "pw": _w((lambda *s: _rng.normal(s) * 0.05)(C, C)),
    }

def reference(x, dw, pw):
    B, H, W, C = x.shape
    k = dw.shape[0]
    pad = k // 2
    xp = jnp.pad(x, ((0,0),(pad,pad),(pad,pad),(0,0)))
    out = jnp.zeros_like(x)
    for i in range(k):
        for j in range(k):
            out = out + xp[:, i:i+H, j:j+W, :] * dw[i, j][None, None, None, :]
    return jnp.einsum('bhwc,cd->bhwd', out, pw)
```

```python
import jax
import jax.numpy as jnp
import jax.experimental.pallas as pl
import jax.experimental.pallas.tpu as pltpu

ROWS = 32
K = 32
SUB = 16
JSTAR = 17


@jax.jit
def pallas_standalone__depthwise_separable__vision_kernel(
    x: jax.Array,
    dw: jax.Array,
    pw: jax.Array,
):
    B, H, W, C = x.shape
    assert dw.shape == (1, 1, C) and pw.shape == (C, C)
    M = B * H * W
    G = M // (K * ROWS)
    assert G * K * ROWS == M and G % SUB == 0

    def kernel_function(x_hbm, dw_ref, pw_ref, o_hbm, buf, rsem, wsem):
        def rd(j):
            return pltpu.make_async_copy(x_hbm.at[:, j], buf.at[j], rsem.at[j])

        def wr(j):
            return pltpu.make_async_copy(buf.at[j], o_hbm.at[:, j], wsem.at[j])

        def compute(j):
            def body(s, carry):
                rows = pl.ds(s * SUB, SUB)
                xs = buf[j, rows].reshape(SUB * ROWS, C) * dw_ref[...]
                y = jnp.dot(xs, pw_ref[...], preferred_element_type=jnp.float32)
                buf[j, rows] = y.astype(buf.dtype).reshape(SUB, ROWS, C)
                return carry

            jax.lax.fori_loop(0, G // SUB, body, 0)

        for j in range(K):
            rd(j).start()

        def phase1(j, carry):
            rd(j).wait()
            compute(j)
            return carry

        jax.lax.fori_loop(0, JSTAR, phase1, 0)

        for j in range(JSTAR, K):
            rd(j).wait()
        for j in range(JSTAR):
            wr(j).start()

        def phase2(j, carry):
            compute(j)
            wr(j).start()
            return carry

        jax.lax.fori_loop(JSTAR, K, phase2, 0)

        for j in range(K):
            wr(j).wait()

    out = pl.pallas_call(
        kernel_function,
        in_specs=[
            pl.BlockSpec(memory_space=pl.ANY),
            pl.BlockSpec(memory_space=pltpu.VMEM),
            pl.BlockSpec(memory_space=pltpu.VMEM),
        ],
        out_specs=pl.BlockSpec(memory_space=pl.ANY),
        out_shape=jax.ShapeDtypeStruct((G, K, ROWS, C), x.dtype),
        scratch_shapes=[
            pltpu.VMEM((K, G, ROWS, C), x.dtype),
            pltpu.SemaphoreType.DMA((K,)),
            pltpu.SemaphoreType.DMA((K,)),
        ],
        compiler_params=pltpu.CompilerParams(vmem_limit_bytes=124 * 1024 * 1024),
    )(x.reshape(G, K, ROWS, C), dw.reshape(1, C), pw)
    return out.reshape(B, H, W, C)
```

```python
import jax
import jax.numpy as jnp
import jax.experimental.pallas as pl
import jax.experimental.pallas.tpu as pltpu

G = 6
R = 768
WR = 48
JSTAR = 18
TAIL = 96
BURST = 16
PACE = 5


@jax.jit
def pallas_standalone__depthwise_separable__vision_kernel(
    x: jax.Array,
    dw: jax.Array,
    pw: jax.Array,
):
    B, H, W, C = x.shape
    assert dw.shape == (1, 1, C) and pw.shape == (C, C)
    M = B * H * W
    S = M // G
    K = S // R
    NW = S // WR
    assert G * S == M and K * R == S and R % WR == 0 and JSTAR < K
    for t in range((K - JSTAR) * G):
        assert BURST + (t + 1) * PACE <= (JSTAR + (t + 1) // G) * (R // WR)

    def kernel_function(
        x_hbm, dw_hbm, pw_hbm, o_hbm, buf, dw_ref, pw_ref, rsem, wsem, psem
    ):
        def read(rows, sem):
            return pltpu.make_async_copy(x_hbm.at[:, rows], buf.at[:, rows], sem)

        def chunk_rows(j):
            return pl.ds(pl.multiple_of(j * R, R), R)

        def read_chunk(j):
            return read(chunk_rows(j), rsem.at[j])

        read_last_head = read(pl.ds(S - R, R - TAIL), rsem.at[K - 1])
        read_last_tail = read(pl.ds(S - TAIL, TAIL), rsem.at[K])

        def start_writes(lo, hi):
            def body(i, carry):
                rows = pl.ds(pl.multiple_of(i * WR, WR), WR)
                pltpu.make_async_copy(buf.at[:, rows], o_hbm.at[:, rows], wsem).start()
                return carry

            jax.lax.fori_loop(lo, hi, body, 0)

        def matmul(j, s):
            rows = chunk_rows(j)
            xs = buf[s, rows] * dw_ref[...]
            y = jnp.dot(xs, pw_ref[...], preferred_element_type=jnp.float32)
            buf[s, rows] = y.astype(buf.dtype)

        read_dw = pltpu.make_async_copy(dw_hbm, dw_ref, psem.at[0])
        read_pw = pltpu.make_async_copy(pw_hbm, pw_ref, psem.at[1])
        read_dw.start()
        read_pw.start()

        def start_read(j, carry):
            read_chunk(j).start()
            return carry

        jax.lax.fori_loop(0, K - 1, start_read, 0)
        read_last_head.start()
        read_last_tail.start()
        read_dw.wait()
        read_pw.wait()

        def read_phase(j, carry):
            read_chunk(j).wait()

            def body(s, c):
                matmul(j, s)
                return c

            return jax.lax.fori_loop(0, G, body, carry)

        jax.lax.fori_loop(0, JSTAR, read_phase, 0)

        for j in range(JSTAR, K - 1):
            read_chunk(j).wait()
        read_last_head.wait()
        start_writes(0, BURST)
        read_last_tail.wait()

        def write_phase(j, carry):
            def body(s, c):
                matmul(j, s)
                lo = BURST + ((j - JSTAR) * G + s) * PACE
                start_writes(lo, lo + PACE)
                return c

            return jax.lax.fori_loop(0, G, body, carry)

        jax.lax.fori_loop(JSTAR, K, write_phase, 0)
        start_writes(BURST + (K - JSTAR) * G * PACE, NW)
        pltpu.make_async_copy(buf, o_hbm, wsem).wait()

    out = pl.pallas_call(
        kernel_function,
        in_specs=[pl.BlockSpec(memory_space=pl.ANY)] * 3,
        out_specs=pl.BlockSpec(memory_space=pl.ANY),
        out_shape=jax.ShapeDtypeStruct((G, S, C), x.dtype),
        scratch_shapes=[
            pltpu.VMEM((G, S, C), x.dtype),
            pltpu.VMEM((1, C), dw.dtype),
            pltpu.VMEM((C, C), pw.dtype),
            pltpu.SemaphoreType.DMA((K + 1,)),
            pltpu.SemaphoreType.DMA(()),
            pltpu.SemaphoreType.DMA((2,)),
        ],
        compiler_params=pltpu.CompilerParams(vmem_limit_bytes=124 * 1024 * 1024),
    )(x.reshape(G, S, C), dw.reshape(1, C), pw)
    return out.reshape(B, H, W, C)
```

```python
import jax
import jax.numpy as jnp
import jax.experimental.pallas as pl
import jax.experimental.pallas.tpu as pltpu

G = 6
R = 768
WR = 48
JSTAR = 17
TAIL = 112
BURST = 24
PACE = 5
SR = 32
NSLOT = 4
AHEAD = 2
EVERY = 5
EXTRA = 1


@jax.jit
def pallas_standalone__depthwise_separable__vision_kernel(
    x: jax.Array,
    dw: jax.Array,
    pw: jax.Array,
):
    B, H, W, C = x.shape
    assert dw.shape == (1, 1, C) and pw.shape == (C, C)
    M = B * H * W
    S = M // G
    K = S // R
    NW = S // WR
    assert G * S == M and K * R == S and NW * WR == S
    for t in range((K - JSTAR) * G):
        assert (BURST + (t + 1) * PACE) * WR <= (JSTAR + (t + 1) // G) * R
    LAG = NSLOT - AHEAD
    NSTEP = pl.cdiv(JSTAR * G, EVERY)
    NSIDE = NSTEP + AHEAD + EXTRA
    SIDE0 = S - NSIDE * SR
    JSIDE = SIDE0 // R
    assert 0 <= EXTRA < LAG <= NSTEP and JSTAR + 1 < JSIDE and SIDE0 % 16 == 0

    def kernel_function(x_hbm, dw_hbm, pw_hbm, o_hbm, buf, dw_ref, pw_ref, ring):
        def body(rsem, hsem, vsem, wsem):
            def read(rows, sem):
                return pltpu.make_async_copy(x_hbm.at[:, rows], buf.at[:, rows], sem)

            def chunk_rows(j):
                return pl.ds(pl.multiple_of(j * R, R), R)

            def read_chunk(j):
                return read(chunk_rows(j), rsem.at[j])

            read_rest = read(pl.ds(JSTAR * R, SIDE0 - TAIL - JSTAR * R), rsem.at[JSTAR])
            read_tail = read(pl.ds(SIDE0 - TAIL, TAIL), rsem.at[JSTAR + 1])
            read_dw = pltpu.make_async_copy(dw_hbm, dw_ref, rsem.at[JSTAR + 2])
            read_pw = pltpu.make_async_copy(pw_hbm, pw_ref, rsem.at[JSTAR + 3])

            def side_rows(i):
                return pl.ds(pl.multiple_of(SIDE0 + i * SR, 16), SR)

            def to_smem(i):
                slot = i % NSLOT
                return pltpu.make_async_copy(
                    x_hbm.at[:, side_rows(i)], ring.at[slot], hsem.at[slot]
                )

            def to_vmem(i):
                slot = i % NSLOT
                return pltpu.make_async_copy(
                    ring.at[slot], buf.at[:, side_rows(i)], vsem.at[slot]
                )

            def side_step(t):
                to_smem(t).wait()
                to_vmem(t).start()

                @pl.when(t >= LAG)
                def _():
                    to_vmem(t - LAG).wait()

                to_smem(t + AHEAD).start()

            def start_writes(lo, hi):
                def start(i, carry):
                    rows = pl.ds(pl.multiple_of(i * WR, WR), WR)
                    pltpu.make_async_copy(
                        buf.at[:, rows], o_hbm.at[:, rows], wsem
                    ).start()
                    return carry

                jax.lax.fori_loop(lo, hi, start, 0)

            def matmul(j, s):
                rows = chunk_rows(j)
                xs = buf[s, rows] * dw_ref[...]
                y = jnp.dot(xs, pw_ref[...], preferred_element_type=jnp.float32)
                buf[s, rows] = y.astype(buf.dtype)

            read_dw.start()
            read_pw.start()
            for i in range(AHEAD):
                to_smem(i).start()

            def start_read(j, carry):
                read_chunk(j).start()
                return carry

            jax.lax.fori_loop(0, JSTAR, start_read, 0)
            read_rest.start()
            read_tail.start()
            read_dw.wait()
            read_pw.wait()

            def read_phase(j, carry):
                read_chunk(j).wait()

                def step(s, c):
                    n = j * G + s

                    @pl.when(n % EVERY == 0)
                    def _():
                        side_step(n // EVERY)

                    matmul(j, s)
                    return c

                return jax.lax.fori_loop(0, G, step, carry)

            jax.lax.fori_loop(0, JSTAR, read_phase, 0)
            for e in range(EXTRA):
                to_vmem(NSTEP - LAG + e).wait()
                to_smem(NSTEP + AHEAD + e).start()

            read_rest.wait()
            start_writes(0, BURST)
            read_tail.wait()

            def write_phase(j, carry):
                @pl.when(j == JSTAR + 1)
                def _():
                    for i in range(NSTEP, NSIDE):
                        to_smem(i).wait()
                        to_vmem(i).start()

                @pl.when(j == JSIDE)
                def _():
                    for i in range(NSTEP - LAG + EXTRA, NSIDE):
                        to_vmem(i).wait()

                def step(s, c):
                    matmul(j, s)
                    lo = BURST + ((j - JSTAR) * G + s) * PACE
                    start_writes(lo, lo + PACE)
                    return c

                return jax.lax.fori_loop(0, G, step, carry)

            jax.lax.fori_loop(JSTAR, K, write_phase, 0)
            start_writes(BURST + (K - JSTAR) * G * PACE, NW)
            pltpu.make_async_copy(buf, o_hbm, wsem).wait()

        pl.run_scoped(
            body,
            pltpu.SemaphoreType.DMA((JSTAR + 4,)),
            pltpu.SemaphoreType.DMA((NSLOT,)),
            pltpu.SemaphoreType.DMA((NSLOT,)),
            pltpu.SemaphoreType.DMA(()),
        )

    out = pl.pallas_call(
        kernel_function,
        in_specs=[pl.BlockSpec(memory_space=pl.ANY)] * 3,
        out_specs=pl.BlockSpec(memory_space=pl.ANY),
        out_shape=jax.ShapeDtypeStruct((G, S, C), x.dtype),
        scratch_shapes=[
            pltpu.VMEM((G, S, C), x.dtype),
            pltpu.VMEM((1, C), dw.dtype),
            pltpu.VMEM((C, C), pw.dtype),
            pltpu.SMEM((NSLOT, G, SR, C), x.dtype),
        ],
        compiler_params=pltpu.CompilerParams(vmem_limit_bytes=124 * 1024 * 1024),
    )(x.reshape(G, S, C), dw.reshape(1, C), pw)
    return out.reshape(B, H, W, C)
```

```python
import jax
import jax.numpy as jnp
import jax.experimental.pallas as pl
import jax.experimental.pallas.tpu as pltpu

G = 6
R = 768
PR = 48
BATCH = 5
DEPTH = 4
PRE = 3
TAIL = 96
BURST = 24
PACE = 5
SG = 2
SR = 112
NSLOT = 3
NCYCLE = 18
CYCLE = 5
VSTEPS = 2
NSEM = 8


@jax.jit
def pallas_standalone__depthwise_separable__vision_kernel(
    x: jax.Array,
    dw: jax.Array,
    pw: jax.Array,
):
    B, H, W, C = x.shape
    assert dw.shape == (1, 1, C) and pw.shape == (C, C)
    M = B * H * W
    S = M // G
    assert G * S == M and S % R == 0 and R % PR == 0 and G % SG == 0
    NSTEP = G * (S // R)
    NSIDE = NCYCLE + NSLOT
    SPLIT = G // SG
    assert NSIDE % SPLIT == 0
    SIDE0 = S - NSIDE // SPLIT * SR
    NB = (SIDE0 - TAIL) // (BATCH * PR)
    NX = (SIDE0 - TAIL) // PR - NB * BATCH
    TAIL0 = (NB * BATCH + NX) * PR
    N1 = NB - 1 - PRE
    NFWD = N1 + G
    NUSE = SIDE0 // R * G
    assert 2 <= DEPTH < NSEM and NCYCLE * CYCLE <= N1 and NFWD < NUSE
    assert NX > 0 and SIDE0 % 16 == 0 and BURST * PR <= N1 // G * R
    for n in range(N1):
        assert (PRE + n + 1) * BATCH * PR >= (n // G + 1) * R

    def kernel_function(x_hbm, dw_hbm, pw_hbm, o_hbm, buf, dw_ref, pw_ref, ring):
        def body(rsem, tsem, hsem, vsem, wsem):
            def loop(lo, hi, fn):
                def step(i, carry):
                    fn(i)
                    return carry

                jax.lax.fori_loop(lo, hi, step, 0)

            def read(row, nrows, sem):
                rows = pl.ds(pl.multiple_of(row, 16), nrows)
                return pltpu.make_async_copy(x_hbm.at[:, rows], buf.at[:, rows], sem)

            def start_batch(b, count=BATCH):
                sem = rsem.at[b & (NSEM - 1)]
                loop(0, count, lambda q: read((b * BATCH + q) * PR, PR, sem).start())

            def wait_batch(b, count=BATCH):
                read(b * (BATCH * PR), count * PR, rsem.at[b & (NSEM - 1)]).wait()

            read_tail = read(TAIL0, SIDE0 - TAIL0, tsem.at[0])
            read_dw = pltpu.make_async_copy(dw_hbm, dw_ref, tsem.at[1])
            read_pw = pltpu.make_async_copy(pw_hbm, pw_ref, tsem.at[2])

            def advance_reads(b):
                wait_batch(b)

                @pl.when(b + DEPTH < NB)
                def _():
                    start_batch(b + DEPTH)

                @pl.when(b + DEPTH == NB)
                def _():
                    start_batch(NB, NX)
                    read_tail.start()

            def side(i):
                rows = pl.ds(pl.multiple_of(SIDE0 + i // SPLIT * SR, 16), SR)
                return pl.ds(i % SPLIT * SG, SG), rows

            def to_smem(i):
                slot = i % NSLOT
                return pltpu.make_async_copy(
                    x_hbm.at[side(i)], ring.at[slot], hsem.at[slot]
                )

            def to_vmem(i):
                slot = i % NSLOT
                return pltpu.make_async_copy(
                    ring.at[slot], buf.at[side(i)], vsem.at[slot]
                )

            def start_write(i):
                rows = pl.ds(pl.multiple_of(i * PR, PR), PR)
                pltpu.make_async_copy(buf.at[:, rows], o_hbm.at[:, rows], wsem).start()

            def matmul(j, s):
                rows = pl.ds(pl.multiple_of(j * R, R), R)
                xs = buf[s, rows] * dw_ref[...]
                y = jnp.dot(xs, pw_ref[...], preferred_element_type=jnp.float32)
                buf[s, rows] = y.astype(buf.dtype)
                wrap = s == G - 1
                return jnp.where(wrap, j + 1, j), jnp.where(wrap, 0, s + 1)

            read_dw.start()
            read_pw.start()
            for i in range(NSLOT - 1):
                to_smem(i).start()
            loop(0, DEPTH, start_batch)
            read_dw.wait()
            read_pw.wait()
            loop(0, PRE, advance_reads)

            def half_cycle(h, js):
                p = h >> 1
                odd = h & 1
                last = h == 2 * NCYCLE

                @pl.when(jnp.logical_and(odd == 0, jnp.logical_not(last)))
                def _():
                    to_smem(p).wait()
                    to_vmem(p).start()

                @pl.when(jnp.logical_or(odd == 1, last))
                def _():
                    @pl.when(p > 0)
                    def _():
                        to_vmem(p - 1).wait()

                    to_smem(p + NSLOT - 1).start()

                def step(n, js):
                    advance_reads(PRE + n)
                    return matmul(*js)

                lo = p * CYCLE + odd * VSTEPS
                hi = p * CYCLE + VSTEPS + odd * (CYCLE - VSTEPS)
                return jax.lax.fori_loop(lo, jnp.where(last, N1, hi), step, js)

            j, s = jax.lax.fori_loop(0, 2 * NCYCLE + 1, half_cycle, (0, 0))
            wait_batch(NB - 1)
            wait_batch(NB, NX)

            loop(0, BURST, start_write)
            read_tail.wait()

            def write_step(n, carry):
                @pl.when(n == NFWD)
                def _():
                    for i in range(NCYCLE, NSIDE):
                        to_smem(i).wait()
                        to_vmem(i).start()

                @pl.when(n == NUSE)
                def _():
                    for i in range(NCYCLE, NSIDE):
                        to_vmem(i).wait()

                j, s, w = carry
                j, s = matmul(j, s)
                w_next = jnp.minimum(w + PACE, j * (R // PR))
                loop(w, w_next, start_write)
                return j, s, w_next

            _, _, w = jax.lax.fori_loop(N1, NSTEP, write_step, (j, s, BURST))
            loop(w, S // PR, start_write)
            pltpu.make_async_copy(buf, o_hbm, wsem).wait()

        pl.run_scoped(
            body,
            pltpu.SemaphoreType.DMA((NSEM,)),
            pltpu.SemaphoreType.DMA((3,)),
            pltpu.SemaphoreType.DMA((NSLOT,)),
            pltpu.SemaphoreType.DMA((NSLOT,)),
            pltpu.SemaphoreType.DMA(()),
        )

    out = pl.pallas_call(
        kernel_function,
        in_specs=[pl.BlockSpec(memory_space=pl.ANY)] * 3,
        out_specs=pl.BlockSpec(memory_space=pl.ANY),
        out_shape=jax.ShapeDtypeStruct((G, S, C), x.dtype),
        scratch_shapes=[
            pltpu.VMEM((G, S, C), x.dtype),
            pltpu.VMEM((1, C), dw.dtype),
            pltpu.VMEM((C, C), pw.dtype),
            pltpu.SMEM((NSLOT, SG, SR, C), x.dtype),
        ],
        compiler_params=pltpu.CompilerParams(vmem_limit_bytes=124 * 1024 * 1024),
    )(x.reshape(G, S, C), dw.reshape(1, C), pw)
    return out.reshape(B, H, W, C)
```

```python
import jax
import jax.numpy as jnp
import jax.experimental.pallas as pl
import jax.experimental.pallas.tpu as pltpu

G = 6
LOG_SB = 12
CH = 256
MG = 3
RUNS = (48, 48, 32)
DEPTH = 4
TAIL = 96
BURST = 8
PACE = 2
SG = 3
SR = 80
NSLOT = 3
NCYCLE = 17
LEAD = 3
CYCLE = 5
VSTEPS = 2
NSEM = 8


@jax.jit
def pallas_standalone__depthwise_separable__vision_kernel(
    x: jax.Array,
    dw: jax.Array,
    pw: jax.Array,
):
    B, H, W, C = x.shape
    assert dw.shape == (1, 1, C) and pw.shape == (C, C)
    SB = 1 << LOG_SB
    U = B * H * W // (G * SB)
    S = U * SB
    UNIT = sum(RUNS)
    assert G * S == B * H * W and SB % CH == 0 and CH % UNIT == 0 and G == 2 * MG
    NSTEP = 2 * (S // CH)
    NSIDE = NCYCLE + NSLOT
    SPLIT = G // SG
    SIDE0 = S - NSIDE // SPLIT * SR
    TAIL0 = SIDE0 - TAIL
    NC = TAIL0 // CH
    NX = TAIL0 % CH // UNIT
    N1 = NC - 1
    NFWD = N1 + 6
    NUSE = 2 * (SIDE0 // CH)
    assert NSIDE % SPLIT == 0 and TAIL0 % UNIT == 0 and TAIL0 >= S - SB and NX > 0
    assert 2 <= DEPTH < NSEM and LEAD + NCYCLE * CYCLE <= N1 and NFWD < NUSE
    assert BURST * UNIT <= N1 // 2 * CH

    def kernel_function(x_hbm, dw_hbm, pw_hbm, o_hbm, buf, dw_ref, pw_ref, ring):
        def body(rsem, tsem, hsem, vsem, wsem):
            def loop(lo, hi, fn):
                def step(i, carry):
                    fn(i)
                    return carry

                jax.lax.fori_loop(lo, hi, step, 0)

            def at(v, n, streams=slice(None)):
                rows = pl.ds(pl.multiple_of(v & (SB - 1), 8), n)
                return v >> LOG_SB, streams, rows

            def unit_runs(v):
                return [at(v + sum(RUNS[:q]), n) for q, n in enumerate(RUNS)]

            def read(idx, sem):
                return pltpu.make_async_copy(x_hbm.at[idx], buf.at[idx], sem)

            def start_chunk(c, units=CH // UNIT):
                for q in range(units):
                    for idx in unit_runs(c * CH + q * UNIT):
                        read(idx, rsem.at[c & (NSEM - 1)]).start()

            def wait_chunk(c, units=CH // UNIT):
                read(at(c * CH, units * UNIT), rsem.at[c & (NSEM - 1)]).wait()

            read_tail = read(at(TAIL0, TAIL), tsem.at[0])
            read_dw = pltpu.make_async_copy(dw_hbm, dw_ref, tsem.at[1])
            read_pw = pltpu.make_async_copy(pw_hbm, pw_ref, tsem.at[2])

            def side(i):
                return at(SIDE0 + i // SPLIT * SR, SR, pl.ds(i % SPLIT * SG, SG))

            def to_smem(i):
                slot = i % NSLOT
                return pltpu.make_async_copy(
                    x_hbm.at[side(i)], ring.at[slot], hsem.at[slot]
                )

            def to_vmem(i):
                slot = i % NSLOT
                return pltpu.make_async_copy(
                    ring.at[slot], buf.at[side(i)], vsem.at[slot]
                )

            def start_write(w):
                for idx in unit_runs(w * UNIT):
                    pltpu.make_async_copy(buf.at[idx], o_hbm.at[idx], wsem).start()

            def matmul(n):
                idx = at((n >> 1) * CH, CH, pl.ds((n & 1) * MG, MG))
                xs = buf[idx].reshape(MG * CH, C) * dw_ref[...]
                y = jnp.dot(xs, pw_ref[...], preferred_element_type=jnp.float32)
                buf[idx] = y.astype(buf.dtype).reshape(MG, CH, C)

            read_dw.start()
            read_pw.start()
            for i in range(NSLOT - 1):
                to_smem(i).start()
            loop(0, DEPTH, start_chunk)
            read_dw.wait()
            read_pw.wait()

            def read_step(n):
                wait_chunk(n)

                @pl.when(n + DEPTH < NC)
                def _():
                    start_chunk(n + DEPTH)

                @pl.when(n + DEPTH == NC)
                def _():
                    start_chunk(NC, NX)
                    read_tail.start()

                matmul(n)

            def half_cycle(h):
                p = h >> 1
                odd = h & 1
                last = h == 2 * NCYCLE

                @pl.when(jnp.logical_and(odd == 0, jnp.logical_not(last)))
                def _():
                    to_smem(p).wait()
                    to_vmem(p).start()

                @pl.when(jnp.logical_and(h > 0, jnp.logical_or(odd == 1, last)))
                def _():
                    @pl.when(p > 0)
                    def _():
                        to_vmem(p - 1).wait()

                    to_smem(p + NSLOT - 1).start()

                lo = LEAD + p * CYCLE + odd * VSTEPS
                hi = LEAD + p * CYCLE + VSTEPS + odd * (CYCLE - VSTEPS)
                loop(jnp.where(h < 0, 0, lo), jnp.where(last, N1, hi), read_step)

            loop(-1, 2 * NCYCLE + 1, half_cycle)
            wait_chunk(NC - 1)
            wait_chunk(NC, NX)

            loop(0, BURST, start_write)
            read_tail.wait()

            def write_step(n, w):
                @pl.when(n == NFWD)
                def _():
                    for i in range(NCYCLE, NSIDE):
                        to_smem(i).wait()
                        to_vmem(i).start()

                @pl.when(n == NUSE)
                def _():
                    for i in range(NCYCLE, NSIDE):
                        to_vmem(i).wait()

                matmul(n)
                w_next = jnp.minimum(w + PACE, ((n + 1) >> 1) * (CH // UNIT))
                loop(w, w_next, start_write)
                return w_next

            w = jax.lax.fori_loop(N1, NSTEP, write_step, BURST)
            loop(w, S // UNIT, start_write)
            pltpu.make_async_copy(buf, o_hbm, wsem).wait()

        pl.run_scoped(
            body,
            pltpu.SemaphoreType.DMA((NSEM,)),
            pltpu.SemaphoreType.DMA((3,)),
            pltpu.SemaphoreType.DMA((NSLOT,)),
            pltpu.SemaphoreType.DMA((NSLOT,)),
            pltpu.SemaphoreType.DMA(()),
        )

    out = pl.pallas_call(
        kernel_function,
        in_specs=[pl.BlockSpec(memory_space=pl.ANY)] * 3,
        out_specs=pl.BlockSpec(memory_space=pl.ANY),
        out_shape=jax.ShapeDtypeStruct((U, G, SB, C), x.dtype),
        scratch_shapes=[
            pltpu.VMEM((U, G, SB, C), x.dtype),
            pltpu.VMEM((1, C), dw.dtype),
            pltpu.VMEM((C, C), pw.dtype),
            pltpu.SMEM((NSLOT, SG, SR, C), x.dtype),
        ],
        compiler_params=pltpu.CompilerParams(vmem_limit_bytes=124 * 1024 * 1024),
    )(x.reshape(U, G, SB, C), dw.reshape(1, C), pw)
    return out.reshape(B, H, W, C)
```

```python
import jax
import jax.numpy as jnp
import jax.experimental.pallas as pl
import jax.experimental.pallas.tpu as pltpu

G = 6
LOG_SB = 12
CH = 256
MG = 3
RUNS = (48, 48, 32)
WRUNS = (48, 48, 32)
DEPTH = 4
TAIL = 96
BURST = 8
PACE = 2
SG = 3
SR = 80
NSLOT = 3
NCYCLE = 17
LEAD = 3
CYCLE = 5
VSTEPS = 2
NSEM = 8


@jax.jit
def pallas_standalone__depthwise_separable__vision_kernel(
    x: jax.Array,
    dw: jax.Array,
    pw: jax.Array,
):
    B, H, W, C = x.shape
    assert dw.shape == (1, 1, C) and pw.shape == (C, C)
    SB = 1 << LOG_SB
    U = B * H * W // (G * SB)
    S = U * SB
    UNIT, WUNIT = sum(RUNS), sum(WRUNS)
    assert G * S == B * H * W and SB % CH == 0 and G == 2 * MG
    assert CH % UNIT == 0 and CH % WUNIT == 0
    NSTEP = 2 * (S // CH)
    NSIDE = NCYCLE + NSLOT
    SPLIT = G // SG
    SIDE0 = S - NSIDE // SPLIT * SR
    TAIL0 = SIDE0 - TAIL
    NC = TAIL0 // CH
    NX = TAIL0 % CH // UNIT
    N1 = NC - 1
    NFWD = N1 + 6
    NUSE = 2 * (SIDE0 // CH)
    assert NSIDE % SPLIT == 0 and TAIL0 % UNIT == 0 and TAIL0 >= S - SB and NX > 0
    assert 2 <= DEPTH < NSEM and LEAD + NCYCLE * CYCLE <= N1 and NFWD < NUSE
    assert BURST * WUNIT <= N1 // 2 * CH
    assert all(n % 16 == 0 for n in RUNS + WRUNS + (SR, TAIL))

    def kernel_function(x_hbm, dw_hbm, pw_hbm, o_hbm, buf, dw_ref, pw_ref, ring):
        def body(rsem, tsem, hsem, vsem, wsem):
            def loop(lo, hi, fn):
                def step(i, carry):
                    fn(i)
                    return carry

                jax.lax.fori_loop(lo, hi, step, 0)

            def at(v, n, streams=slice(None)):
                rows = pl.ds(pl.multiple_of(v & (SB - 1), 16), n)
                return v >> LOG_SB, streams, rows

            def split(v, runs):
                return [at(v + sum(runs[:q]), n) for q, n in enumerate(runs)]

            def read(idx, sem):
                return pltpu.make_async_copy(x_hbm.at[idx], buf.at[idx], sem)

            def start_chunk(c, units=CH // UNIT):
                for idx in split(c * CH, RUNS * units):
                    read(idx, rsem.at[c & (NSEM - 1)]).start()

            def wait_chunk(c, units=CH // UNIT):
                read(at(c * CH, units * UNIT), rsem.at[c & (NSEM - 1)]).wait()

            read_tail = read(at(TAIL0, TAIL), tsem.at[0])
            read_dw = pltpu.make_async_copy(dw_hbm, dw_ref, tsem.at[1])
            read_pw = pltpu.make_async_copy(pw_hbm, pw_ref, tsem.at[2])

            def side(i):
                return at(SIDE0 + i // SPLIT * SR, SR, pl.ds(i % SPLIT * SG, SG))

            def to_smem(i):
                slot = i % NSLOT
                return pltpu.make_async_copy(
                    x_hbm.at[side(i)], ring.at[slot], hsem.at[slot]
                )

            def to_vmem(i):
                slot = i % NSLOT
                return pltpu.make_async_copy(
                    ring.at[slot], buf.at[side(i)], vsem.at[slot]
                )

            def start_write(w):
                for idx in split(w * WUNIT, WRUNS):
                    pltpu.make_async_copy(buf.at[idx], o_hbm.at[idx], wsem).start()

            def matmul(n):
                idx = at((n >> 1) * CH, CH, pl.ds((n & 1) * MG, MG))
                xs = buf[idx].reshape(MG * CH, C) * dw_ref[...]
                y = jnp.dot(xs, pw_ref[...], preferred_element_type=jnp.float32)
                buf[idx] = y.astype(buf.dtype).reshape(MG, CH, C)

            read_dw.start()
            read_pw.start()
            for i in range(NSLOT - 1):
                to_smem(i).start()
            loop(0, DEPTH, start_chunk)
            read_dw.wait()
            read_pw.wait()

            def read_step(n):
                wait_chunk(n)

                @pl.when(n + DEPTH < NC)
                def _():
                    start_chunk(n + DEPTH)

                @pl.when(n + DEPTH == NC)
                def _():
                    start_chunk(NC, NX)
                    read_tail.start()

                matmul(n)

            def half_cycle(h):
                p = h >> 1
                odd = h & 1
                last = h == 2 * NCYCLE

                @pl.when(jnp.logical_and(odd == 0, jnp.logical_not(last)))
                def _():
                    to_smem(p).wait()
                    to_vmem(p).start()

                @pl.when(jnp.logical_and(h > 0, jnp.logical_or(odd == 1, last)))
                def _():
                    @pl.when(p > 0)
                    def _():
                        to_vmem(p - 1).wait()

                    to_smem(p + NSLOT - 1).start()

                lo = LEAD + p * CYCLE + odd * VSTEPS
                hi = LEAD + p * CYCLE + VSTEPS + odd * (CYCLE - VSTEPS)
                loop(jnp.where(h < 0, 0, lo), jnp.where(last, N1, hi), read_step)

            loop(-1, 2 * NCYCLE + 1, half_cycle)
            wait_chunk(NC - 1)
            wait_chunk(NC, NX)

            loop(0, BURST, start_write)
            read_tail.wait()

            def write_step(n, w):
                @pl.when(n == NFWD)
                def _():
                    for i in range(NCYCLE, NSIDE):
                        to_smem(i).wait()
                        to_vmem(i).start()

                @pl.when(n == NUSE)
                def _():
                    for i in range(NCYCLE, NSIDE):
                        to_vmem(i).wait()

                matmul(n)
                w_next = jnp.minimum(w + PACE, ((n + 1) >> 1) * (CH // WUNIT))
                loop(w, w_next, start_write)
                return w_next

            w = jax.lax.fori_loop(N1, NSTEP, write_step, BURST)
            loop(w, S // WUNIT, start_write)
            pltpu.make_async_copy(buf, o_hbm, wsem).wait()

        pl.run_scoped(
            body,
            pltpu.SemaphoreType.DMA((NSEM,)),
            pltpu.SemaphoreType.DMA((3,)),
            pltpu.SemaphoreType.DMA((NSLOT,)),
            pltpu.SemaphoreType.DMA((NSLOT,)),
            pltpu.SemaphoreType.DMA(()),
        )

    out = pl.pallas_call(
        kernel_function,
        in_specs=[pl.BlockSpec(memory_space=pl.ANY)] * 3,
        out_specs=pl.BlockSpec(memory_space=pl.ANY),
        out_shape=jax.ShapeDtypeStruct((U, G, SB, C), x.dtype),
        scratch_shapes=[
            pltpu.VMEM((U, G, SB, C), x.dtype),
            pltpu.VMEM((1, C), dw.dtype),
            pltpu.VMEM((C, C), pw.dtype),
            pltpu.SMEM((NSLOT, SG, SR, C), x.dtype),
        ],
        compiler_params=pltpu.CompilerParams(vmem_limit_bytes=124 * 1024 * 1024),
    )(x.reshape(U, G, SB, C), dw.reshape(1, C), pw)
    return out.reshape(B, H, W, C)
```

```python
import jax
import jax.numpy as jnp
import jax.experimental.pallas as pl
import jax.experimental.pallas.tpu as pltpu

G = 6
LOG_SB = 12
CH = 256
MG = 3
RUNS = (48, 32, 48)
WRUNS = (48, 48, 32)
DEPTH = 4
TAIL = 96
BURST = 10
PACE = 2
SG = 3
SR = 80
NSLOT = 3
NCYCLE = 17
LEAD = 3
CYCLE = 5
VSTEPS = 2
NSEM = 8
NEARLY = 17
ER = 64
ALIGN = 16


@jax.jit
def pallas_standalone__depthwise_separable__vision_kernel(
    x: jax.Array,
    dw: jax.Array,
    pw: jax.Array,
):
    B, H, W, C = x.shape
    assert dw.shape == (1, 1, C) and pw.shape == (C, C)
    SB = 1 << LOG_SB
    U = B * H * W // (G * SB)
    S = U * SB
    UNIT, WUNIT = sum(RUNS), sum(WRUNS)
    assert G * S == B * H * W and SB % CH == 0 and G == 2 * MG
    assert CH % UNIT == 0 and CH % WUNIT == 0
    NSTEP = 2 * (S // CH)
    NSIDE = NCYCLE + NSLOT
    SPLIT = G // SG
    SIDE0 = S - NSIDE // SPLIT * SR
    TAIL0 = SIDE0 - TAIL
    NC = TAIL0 // CH
    NX = TAIL0 % CH // UNIT
    N1 = NC - 1
    NFWD = N1 + 6
    NUSE = 2 * (SIDE0 // CH)
    assert NSIDE % SPLIT == 0 and TAIL0 % UNIT == 0 and TAIL0 >= S - SB and NX > 0
    assert 2 <= DEPTH < NSEM and LEAD + NCYCLE * CYCLE <= N1 and NFWD < NUSE
    assert BURST * WUNIT <= N1 // 2 * CH
    EARLY = pl.cdiv(NEARLY, G) * ER
    W0 = pl.cdiv(EARLY, WUNIT)
    assert NEARLY <= NCYCLE and EARLY <= CH and LEAD >= 2 and W0 < BURST
    assert all(n % ALIGN == 0 for n in RUNS + WRUNS + (SR, TAIL, ER))

    def kernel_function(x_hbm, dw_hbm, pw_hbm, o_hbm, buf, dw_ref, pw_ref, ring):
        def body(rsem, tsem, hsem, vsem, wsem):
            def loop(lo, hi, fn):
                def step(i, carry):
                    fn(i)
                    return carry

                jax.lax.fori_loop(lo, hi, step, 0)

            def at(v, n, streams=slice(None)):
                rows = pl.ds(pl.multiple_of(v & (SB - 1), ALIGN), n)
                return v >> LOG_SB, streams, rows

            def split(v, runs):
                return [at(v + sum(runs[:q]), n) for q, n in enumerate(runs)]

            def read(idx, sem):
                return pltpu.make_async_copy(x_hbm.at[idx], buf.at[idx], sem)

            def start_chunk(c, units=CH // UNIT):
                for idx in split(c * CH, RUNS * units):
                    read(idx, rsem.at[c & (NSEM - 1)]).start()

            def wait_chunk(c, units=CH // UNIT):
                read(at(c * CH, units * UNIT), rsem.at[c & (NSEM - 1)]).wait()

            read_tail = read(at(TAIL0, TAIL), tsem.at[0])
            read_dw = pltpu.make_async_copy(dw_hbm, dw_ref, tsem.at[1])
            read_pw = pltpu.make_async_copy(pw_hbm, pw_ref, tsem.at[2])

            def side(i):
                return at(SIDE0 + i // SPLIT * SR, SR, pl.ds(i % SPLIT * SG, SG))

            def to_smem(i):
                slot = i % NSLOT
                return pltpu.make_async_copy(
                    x_hbm.at[side(i)], ring.at[slot], hsem.at[slot]
                )

            def to_vmem(i):
                slot = i % NSLOT
                return pltpu.make_async_copy(
                    ring.at[slot], buf.at[side(i)], vsem.at[slot]
                )

            def write(idx):
                pltpu.make_async_copy(buf.at[idx], o_hbm.at[idx], wsem).start()

            def start_write(w):
                for idx in split(w * WUNIT, WRUNS):
                    write(idx)

            def matmul(n):
                idx = at((n >> 1) * CH, CH, pl.ds((n & 1) * MG, MG))
                xs = buf[idx].reshape(MG * CH, C) * dw_ref[...]
                y = jnp.dot(xs, pw_ref[...], preferred_element_type=jnp.float32)
                buf[idx] = y.astype(buf.dtype).reshape(MG, CH, C)

            read_dw.start()
            read_pw.start()
            for i in range(NSLOT - 1):
                to_smem(i).start()
            loop(0, DEPTH, start_chunk)
            read_dw.wait()
            read_pw.wait()

            def read_step(n, p):
                wait_chunk(n)

                @pl.when(n + DEPTH < NC)
                def _():
                    start_chunk(n + DEPTH)

                @pl.when(n + DEPTH == NC)
                def _():
                    start_chunk(NC, NX)
                    read_tail.start()

                first = jnp.logical_and(n == LEAD + p * CYCLE, p >= 0)

                @pl.when(jnp.logical_and(first, p < NEARLY))
                def _():
                    write(at(p // G * ER, ER, pl.ds(p % G, 1)))

                matmul(n)

            def half_cycle(h):
                p = h >> 1
                odd = h & 1
                last = h == 2 * NCYCLE

                @pl.when(jnp.logical_and(odd == 0, jnp.logical_not(last)))
                def _():
                    to_smem(p).wait()
                    to_vmem(p).start()

                @pl.when(jnp.logical_and(h > 0, jnp.logical_or(odd == 1, last)))
                def _():
                    @pl.when(p > 0)
                    def _():
                        to_vmem(p - 1).wait()

                    to_smem(p + NSLOT - 1).start()

                lo = LEAD + p * CYCLE + odd * VSTEPS
                hi = LEAD + p * CYCLE + VSTEPS + odd * (CYCLE - VSTEPS)
                lo, hi = jnp.where(h < 0, 0, lo), jnp.where(last, N1, hi)
                loop(lo, hi, lambda n: read_step(n, p))

            loop(-1, 2 * NCYCLE + 1, half_cycle)
            wait_chunk(NC - 1)
            wait_chunk(NC, NX)

            if NEARLY % G:
                write(at(EARLY - ER, ER, pl.ds(NEARLY % G, G - NEARLY % G)))
            if W0 * WUNIT > EARLY:
                write(at(EARLY, W0 * WUNIT - EARLY))
            loop(W0, BURST, start_write)
            read_tail.wait()

            def write_step(n, w):
                @pl.when(n == NFWD)
                def _():
                    for i in range(NCYCLE, NSIDE):
                        to_smem(i).wait()
                        to_vmem(i).start()

                @pl.when(n == NUSE)
                def _():
                    for i in range(NCYCLE, NSIDE):
                        to_vmem(i).wait()

                matmul(n)
                w_next = jnp.minimum(w + PACE, ((n + 1) >> 1) * (CH // WUNIT))
                loop(w, w_next, start_write)
                return w_next

            w = jax.lax.fori_loop(N1, NSTEP, write_step, BURST)
            loop(w, S // WUNIT, start_write)
            pltpu.make_async_copy(buf, o_hbm, wsem).wait()

        pl.run_scoped(
            body,
            pltpu.SemaphoreType.DMA((NSEM,)),
            pltpu.SemaphoreType.DMA((3,)),
            pltpu.SemaphoreType.DMA((NSLOT,)),
            pltpu.SemaphoreType.DMA((NSLOT,)),
            pltpu.SemaphoreType.DMA(()),
        )

    out = pl.pallas_call(
        kernel_function,
        in_specs=[pl.BlockSpec(memory_space=pl.ANY)] * 3,
        out_specs=pl.BlockSpec(memory_space=pl.ANY),
        out_shape=jax.ShapeDtypeStruct((U, G, SB, C), x.dtype),
        scratch_shapes=[
            pltpu.VMEM((U, G, SB, C), x.dtype),
            pltpu.VMEM((1, C), dw.dtype),
            pltpu.VMEM((C, C), pw.dtype),
            pltpu.SMEM((NSLOT, SG, SR, C), x.dtype),
        ],
        compiler_params=pltpu.CompilerParams(vmem_limit_bytes=124 * 1024 * 1024),
    )(x.reshape(U, G, SB, C), dw.reshape(1, C), pw)
    return out.reshape(B, H, W, C)
```
